```python
import os as _os
_os.environ.setdefault("JAX_PLATFORMS", "cpu")
import jax
import jax.numpy as jnp

def _softmax(x, axis=-1):
    return jax.nn.softmax(x, axis=axis)
def _gelu(x):
    return jax.nn.gelu(x, approximate=True)
def _silu(x):
    return jax.nn.silu(x)
def _sigmoid(x):
    return jax.nn.sigmoid(x)
def _layernorm(x, axis=-1, eps=1e-5):
    m = jnp.mean(x, axis=axis, keepdims=True)
    v = jnp.var(x, axis=axis, keepdims=True)
    return (x - m) / jnp.sqrt(v + eps)
def _scatter_add(tgt, idx, src, axis=0):
    return tgt.at[idx].add(src)
def _segment_sum(src, seg, n):
    return jax.ops.segment_sum(src, seg, n)
class _Rng:
    def __init__(self, key):
        self._k = key
    def _next(self):
        self._k, sub = jax.random.split(self._k)
        return sub
    def normal(self, shape):
        return jax.random.normal(self._next(), shape, dtype=jnp.bfloat16)
    def randint(self, lo, hi, shape):
        return jax.random.randint(self._next(), shape, lo, hi, dtype=jnp.int32)
    def uniform(self, shape, lo=0.0, hi=1.0):
        return jax.random.uniform(self._next(), shape, jnp.bfloat16, lo, hi)
    def permutation(self, n):
        return jax.random.permutation(self._next(), n)


kernel_name = 'sequential_preLN__softmax_full_mha__glu_gated_swiglu__prompt'

def setup_inputs():
    _rng = _Rng(jax.random.key(int.from_bytes(__import__("os").urandom(4), "little")))
    _w = (lambda a: (lambda t: t.astype(jnp.bfloat16) if jnp.issubdtype(t.dtype, jnp.floating) else t)(jnp.asarray(a)))
    def _A_setup():
        B, S, D = 1, 2048, 640
        return {
            "x": _w((lambda *s: _rng.normal(s) * 0.05)(B, S, D)),
            "wqkv": _w((lambda *s: _rng.normal(s) * 0.05)(D, 3 * D)),
            "wo": _w((lambda *s: _rng.normal(s) * 0.05)(D, D)),
        }
    _A_in = _A_setup()

    def _B_setup():
        B, S, D, F = 1, 2048, 640, 1728
        return {
            "x": _w((lambda *s: _rng.normal(s) * 0.05)(B, S, D)),
            "w1": _w((lambda *s: _rng.normal(s) * 0.05)(D, F) * (2.0 / D) ** 0.5),
            "w3": _w((lambda *s: _rng.normal(s) * 0.05)(D, F) * (2.0 / D) ** 0.5),
            "w2": _w((lambda *s: _rng.normal(s) * 0.05)(F, D) * (2.0 / F) ** 0.5),
        }
    _B_in = _B_setup()

    return {
        "A_x": _A_in["x"],
        "A_wqkv": _A_in["wqkv"],
        "A_wo": _A_in["wo"],
        "B_x": _B_in["x"],
        "B_w1": _B_in["w1"],
        "B_w3": _B_in["w3"],
        "B_w2": _B_in["w2"],
    }

def reference(A_x, A_wqkv, A_wo, B_x, B_w1, B_w3, B_w2):
    def _A_ref(x, wqkv, wo):
        B, S, D = x.shape
        H = 32; Dh = D // H
        qkv = (lambda x, *d: x.transpose(*d))((x @ wqkv).reshape(B, S, 3, H, Dh), 2, 0, 3, 1, 4)
        q, k, v = qkv[0], qkv[1], qkv[2]
        scale = Dh ** -0.5
        scores = jnp.einsum("bhqd,bhkd->bhqk", q, k) * scale
        p = _softmax(scores, axis=-1)
        o = jnp.einsum("bhqk,bhkd->bhqd", p, v)
        return (lambda x, *d: x.transpose(*d))(o, 0, 2, 1, 3).reshape(B, S, D) @ wo

    def _B_ref(x, w1, w3, w2):
        gate = jnp.einsum("bsd,df->bsf", x, w1)
        up = jnp.einsum("bsd,df->bsf", x, w3)
        h = _silu(gate) * up
        out = jnp.einsum("bsf,fd->bsd", h, w2)
        return out

    x = A_x
    h = x + _A_ref(_layernorm(x, axis=-1), A_wqkv, A_wo)
    h2 = h + _B_ref(_layernorm(h, axis=-1), B_w1, B_w3, B_w2)
    return h2
```

```python
import functools
import math
import numpy as np
import jax
import jax.numpy as jnp
from jax import lax
import jax.experimental.pallas as pl
import jax.experimental.pallas.tpu as pltpu

S, D, H, DH, F = 2048, 640, 32, 20, 1728
NW = 9
TQ = 512
NS = S // TQ
CK = 128
NC = S // CK
RB = 512
NRB = S // RB
EPS = 1e-5
QSCALE = float(DH ** -0.5 * math.log2(math.e))
NT_DIMS = (((1,), (1,)), ((), ()))
F32, BF16, U32 = jnp.float32, jnp.bfloat16, jnp.uint32


def _ln(x):
    mu = jnp.mean(x, axis=-1, keepdims=True)
    xc = x - mu
    var = jnp.mean(xc * xc, axis=-1, keepdims=True)
    return xc * lax.rsqrt(var + EPS)


def _kernel(x_hbm, wqkv_hbm, wo_hbm, w1t_hbm, w3t_hbm, w2_hbm, o_hbm,
            x_ref, wqkv_ref, wo_ref, w1t_ref, w3t_ref, w2_ref, y_ref,
            wqvt_ref, kw_ref, qt_ref, vt_ref, s_ref, ot_ref, in_sems, out_sems):
    x_copies = [pltpu.make_async_copy(x_hbm.at[pl.ds(r * RB, RB)], x_ref.at[pl.ds(r * RB, RB)], in_sems.at[r])
                for r in range(NRB)]
    wqkv_copy = pltpu.make_async_copy(wqkv_hbm, wqkv_ref, in_sems.at[NRB])
    late_copies = [pltpu.make_async_copy(src, dst, in_sems.at[NRB + 1 + i]) for i, (src, dst) in enumerate(
        [(wo_hbm, wo_ref), (w1t_hbm, w1t_ref), (w3t_hbm, w3t_ref), (w2_hbm, w2_ref)])]
    wqkv_copy.start()
    for cp in x_copies:
        cp.start()
    for cp in late_copies:
        cp.start()

    with jax.named_scope("p0_wait"):
        wqkv_copy.wait()
    with jax.named_scope("p0"):
        wqvt_ref[0:D, :] = wqkv_ref[:, 0:D].T
        wqvt_ref[D:2 * D, :] = wqkv_ref[:, 2 * D:3 * D].T

    lane = lax.broadcasted_iota(jnp.int32, (8, 128), 1)
    lo_half = lane < 64

    def proj(r, carry):
        rows = pl.ds(pl.multiple_of(r * RB, RB), RB)
        prow = pl.ds(pl.multiple_of(r * (RB // 2), RB // 2), RB // 2)
        pltpu.make_async_copy(x_hbm.at[rows], x_ref.at[rows], in_sems.at[r]).wait()
        xn = _ln(x_ref[rows, :].astype(F32)).astype(BF16)
        k = jnp.dot(xn, wqkv_ref[:, D:2 * D], preferred_element_type=F32).astype(BF16)
        ku = pltpu.bitcast(k, U32)
        tiles = [ku[:, t * 128:(t + 1) * 128].reshape(RB // 16, 8, 128) for t in range(5)]
        rolled = [pltpu.roll(t_, 64, 2) for t_ in tiles]
        for t in range(5):
            kw_ref[2 * t, prow, :] = tiles[t].reshape(RB // 2, 128)
        for t in range(4):
            kw_ref[2 * t + 1, prow, :] = jnp.where(lo_half[None], rolled[t], rolled[t + 1]).reshape(RB // 2, 128)
        qv = lax.dot_general(wqvt_ref[...], xn, NT_DIMS, preferred_element_type=F32)
        qt_ref[:, rows] = pltpu.bitcast((qv[0:D] * QSCALE).astype(BF16), U32)
        vt_ref[:, rows] = qv[D:2 * D].astype(BF16).astype(F32)
        return carry
    with jax.named_scope("p1"):
        lax.fori_loop(0, NRB, proj, 0)

    sub64 = lax.broadcasted_iota(jnp.int32, (64, 128), 0)
    row24 = lax.broadcasted_iota(jnp.int32, (24, 128), 0)
    row24q = lax.broadcasted_iota(jnp.int32, (24, TQ), 0)

    def qmask(h, js):
        w = jnp.minimum((h * DH) >> 6, NW - 1)
        lo2 = (h * DH - w * 64) >> 1
        msk = jnp.where((sub64 >= lo2) & (sub64 < lo2 + DH // 2), U32(0xFFFFFFFF), U32(0))
        qi = qt_ref[pl.ds(pl.multiple_of(w * 32, 32), 64), js * TQ:(js + 1) * TQ]
        qi = qi & jnp.concatenate([msk] * (TQ // 128), axis=1)
        return w, pltpu.bitcast(qi, BF16)

    def qk_chunk(w, qm, js, c):
        kc = pltpu.bitcast(kw_ref[w, c * (CK // 2):(c + 1) * (CK // 2), :], BF16)
        s = jnp.dot(kc, qm, preferred_element_type=F32)
        s_ref[js, c * CK:(c + 1) * CK, :] = s
        return jnp.max(s.reshape(CK // 8, 8, TQ), axis=0)

    def pexp(js, c, m_cur):
        return jnp.exp2(s_ref[js, c * CK:(c + 1) * CK, :] - m_cur).astype(BF16)

    def pv_chunk(p, r0, ones_mask, c):
        v = jnp.where(ones_mask, 1.0, vt_ref[pl.ds(r0, 24), c * CK:(c + 1) * CK])
        return jnp.dot(v, p, preferred_element_type=F32)

    def finish(acc, js, r0, off, ones_row):
        l = jnp.sum(jnp.where(row24q == ones_row, acc, 0.0), axis=0, keepdims=True)
        o = acc * (1.0 / l)
        keep = (row24q >= off) & (row24q < off + DH)
        pltpu.store(ot_ref.at[pl.ds(r0, 24), js * TQ:(js + 1) * TQ], o, mask=keep)

    ms = []
    with jax.named_scope("p2_pro"):
        for js in range(NS):
            w, qm = qmask(0, js)
            mx = None
            for c in range(NC):
                mc = qk_chunk(w, qm, js, c)
                mx = mc if mx is None else jnp.maximum(mx, mc)
            ms.append(jnp.max(mx, axis=0, keepdims=True))

    slots = [(js, c) for js in range(NS) for c in range(NC)]

    def head_step(h, ms):
        off = (h & 1) * 4
        r0 = pl.multiple_of(h * DH - off, 8)
        ones_row = jnp.where(off == 0, 20, 0)
        ones_mask = row24 == ones_row
        new_ms = []
        st = {}

        def do_qk(n):
            js, c = slots[n]
            if c == 0:
                st['q'] = qmask(h + 1, js)
                st['mx'] = None
            w, qm = st['q']
            mc = qk_chunk(w, qm, js, c)
            st['mx'] = mc if st['mx'] is None else jnp.maximum(st['mx'], mc)
            if c == NC - 1:
                new_ms.append(jnp.max(st['mx'], axis=0, keepdims=True))

        p_next = pexp(0, 0, ms[0])
        do_qk(0)
        acc = None
        for n, (js, c) in enumerate(slots):
            p = p_next
            if n + 1 < len(slots):
                p_next = pexp(slots[n + 1][0], slots[n + 1][1], ms[slots[n + 1][0]])
                do_qk(n + 1)
            d = pv_chunk(p, r0, ones_mask, c)
            acc = d if c == 0 else acc + d
            if c == NC - 1:
                finish(acc, js, r0, off, ones_row)
        return tuple(new_ms)

    with jax.named_scope("p2_loop"):
        ms = lax.fori_loop(0, H - 1, head_step, tuple(ms))

    h = H - 1
    off = (h & 1) * 4
    r0 = h * DH - off
    ones_row = 20 if off == 0 else 0
    with jax.named_scope("p2_epi"):
        for js in range(NS):
            acc = None
            for c in range(NC):
                d = pv_chunk(pexp(js, c, ms[js]), r0, row24 == ones_row, c)
                acc = d if acc is None else acc + d
            finish(acc, js, r0, off, ones_row)

    with jax.named_scope("p3_wait"):
        for cp in late_copies:
            cp.wait()

    def out_copy(r):
        rows = pl.ds(pl.multiple_of(r * RB, RB), RB)
        return pltpu.make_async_copy(y_ref.at[rows], o_hbm.at[rows], out_sems.at[r])

    def tail(r, c):
        rows = pl.ds(pl.multiple_of(r * RB, RB), RB)
        o = ot_ref[:, rows].astype(BF16).T
        hres = x_ref[rows, :].astype(F32) + jnp.dot(o, wo_ref[...], preferred_element_type=F32)
        hn = _ln(hres).astype(BF16)
        g = lax.dot_general(hn, w1t_ref[...], NT_DIMS, preferred_element_type=F32)
        u = lax.dot_general(hn, w3t_ref[...], NT_DIMS, preferred_element_type=F32)
        a = (g * jax.nn.sigmoid(g) * u).astype(BF16)
        y = hres + jnp.dot(a, w2_ref[...], preferred_element_type=F32)
        y_ref[rows, :] = y.astype(BF16)
        out_copy(r).start()
        return c
    with jax.named_scope("p3"):
        lax.fori_loop(0, NRB, tail, 0)
    with jax.named_scope("p3_out"):
        for r in range(NRB):
            out_copy(r).wait()


@jax.jit
def pallas_sequential_preLN__softmax_full_mha__glu_gated_swiglu__prompt_kernel(
    A_x, A_wqkv, A_wo, B_x, B_w1, B_w3, B_w2,
):
    del B_x
    x = A_x.reshape(S, D)
    hbm = pl.BlockSpec(memory_space=pltpu.HBM)
    out = pl.pallas_call(
        _kernel,
        out_shape=jax.ShapeDtypeStruct((S, D), BF16),
        in_specs=[hbm] * 6,
        out_specs=hbm,
        scratch_shapes=[
            pltpu.VMEM((S, D), BF16),
            pltpu.VMEM((D, 3 * D), BF16),
            pltpu.VMEM((D, D), BF16),
            pltpu.VMEM((F, D), BF16),
            pltpu.VMEM((F, D), BF16),
            pltpu.VMEM((F, D), BF16),
            pltpu.VMEM((S, D), BF16),
            pltpu.VMEM((2 * D, D), BF16),
            pltpu.VMEM((NW, S // 2, 128), U32),
            pltpu.VMEM((D // 2, S), U32),
            pltpu.VMEM((D, S), F32),
            pltpu.VMEM((NS, S, TQ), F32),
            pltpu.VMEM((D, S), F32),
            pltpu.SemaphoreType.DMA((NRB + 5,)),
            pltpu.SemaphoreType.DMA((NRB,)),
        ],
        compiler_params=pltpu.CompilerParams(vmem_limit_bytes=110 * 1024 * 1024),
        name="fused_block",
    )(x, A_wqkv, A_wo, B_w1.T, B_w3.T, B_w2)
    return out.reshape(1, S, D)
```

```python
import math

import jax
import jax.numpy as jnp
from jax import lax
import jax.experimental.pallas as pl
import jax.experimental.pallas.tpu as pltpu

S, D, H, DH, F = 2048, 640, 32, 20, 1728
NW = 9
TQ = 512
NS = S // TQ
CK = 128
NC = S // CK
RB = 512
NRB = S // RB
HR = RB // 2
FM = 1664
FT = F - FM
LNG = 16
EPS = 1e-5
GROUPS = ((0, 4), (4, 3), (7, 3), (10, 3))
QSCALE = float(DH ** -0.5 * math.log2(math.e))
NT_DIMS = (((1,), (1,)), ((), ()))
F32, BF16, U32 = jnp.float32, jnp.bfloat16, jnp.uint32


def _ln(x):
    mu = jnp.mean(x, axis=-1, keepdims=True)
    xc = x - mu
    var = jnp.mean(xc * xc, axis=-1, keepdims=True)
    return xc * lax.rsqrt(var + EPS)


def _silu(g):
    return g * jax.nn.sigmoid(g)


def _kernel(x_hbm, wqkv_hbm, wo_hbm, w1t_hbm, w3t_hbm, w2_hbm, o_hbm,
            x_ref, wqkv_ref, wo_ref, w13t_ref, w2_ref, y_ref,
            xn_ref, wqvt_ref, kw_ref, qt_ref, vt_ref, s_ref, ot_ref, m_ref, acc_ref, ob_ref,
            x_sems, w_sems, out_sems):
    def blk(r):
        return pl.ds(r * RB if isinstance(r, int) else pl.multiple_of(r * RB, RB), RB)

    def x_copy(r):
        return pltpu.make_async_copy(x_hbm.at[blk(r)], x_ref.at[blk(r)], x_sems.at[r])

    wk_copy = pltpu.make_async_copy(wqkv_hbm.at[:, D:2 * D], wqkv_ref.at[:, D:2 * D], w_sems.at[0])
    wq_copy = pltpu.make_async_copy(wqkv_hbm.at[:, 0:D], wqkv_ref.at[:, 0:D], w_sems.at[1])
    wv_copy = pltpu.make_async_copy(wqkv_hbm.at[:, 2 * D:3 * D], wqkv_ref.at[:, 2 * D:3 * D], w_sems.at[2])
    late_copies = [
        pltpu.make_async_copy(wo_hbm, wo_ref, w_sems.at[3]),
        pltpu.make_async_copy(w1t_hbm.at[0:FM], w13t_ref.at[0:FM], w_sems.at[4]),
        pltpu.make_async_copy(w3t_hbm.at[0:FM], w13t_ref.at[FM:2 * FM], w_sems.at[5]),
        pltpu.make_async_copy(w1t_hbm.at[FM:F], w13t_ref.at[2 * FM:2 * FM + FT], w_sems.at[6]),
        pltpu.make_async_copy(w3t_hbm.at[FM:F], w13t_ref.at[2 * FM + FT:2 * F], w_sems.at[7]),
        pltpu.make_async_copy(w2_hbm, w2_ref.at[0:F], w_sems.at[8]),
    ]
    x_copy(0).start()
    wk_copy.start()
    x_copy(1).start()
    x_copy(2).start()
    x_copy(3).start()
    wq_copy.start()
    wv_copy.start()

    lane = lax.broadcasted_iota(jnp.int32, (8, 128), 1)
    lo_half = lane < 64

    def ln_block(r):
        for g in range(RB // LNG):
            rows = pl.ds(r * RB + g * LNG, LNG)
            prows = pl.ds(r * (RB // 2) + g * (LNG // 2), LNG // 2)
            xn_ref[prows, :] = pltpu.bitcast(_ln(x_ref[rows, :].astype(F32)).astype(BF16), U32)

    def kproj(r):
        for i in range(4):
            prow = pl.ds(r * (RB // 2) + i * (RB // 8), RB // 8)
            k = jnp.dot(pltpu.bitcast(xn_ref[prow, :], BF16), wqkv_ref[:, D:2 * D], preferred_element_type=F32)
            ku = pltpu.bitcast(k.astype(BF16), U32)
            for t in range(5):
                kw_ref[2 * t, prow, :] = ku[:, t * 128:(t + 1) * 128]

    with jax.named_scope("ln_kproj"):
        x_copy(0).wait()
        ln_block(0)
        w2_ref[F:F + FT, :] = jnp.zeros((FT, D), BF16)
        wk_copy.wait()
        kproj(0)
        x_copy(1).wait()
        x_copy(2).wait()
        ln_block(1)
        kproj(1)
        ln_block(2)
        x_copy(3).wait()
        wq_copy.wait()
        wv_copy.wait()
        for cp in late_copies:
            cp.start()
        kproj(2)
        ln_block(3)
        kproj(3)
        wqvt_ref[0:D, :] = wqkv_ref[:, 0:D].T
        wqvt_ref[D:2 * D, :] = wqkv_ref[:, 2 * D:3 * D].T

    row24 = lax.broadcasted_iota(jnp.int32, (24, 128), 0)
    row24q = lax.broadcasted_iota(jnp.int32, (24, TQ), 0)

    def cols(js):
        return pl.ds(js * TQ if isinstance(js, int) else pl.multiple_of(js * TQ, TQ), TQ)

    def window(h):
        return jnp.minimum((h * DH) >> 6, NW - 1)

    def kmask(h, c):
        w = window(h)
        lo = h * DH - w * 64
        lm = jnp.where((lane >= lo) & (lane < lo + DH), U32(0xFFFFFFFF), U32(0))
        ki = kw_ref[w, c * (CK // 2):(c + 1) * (CK // 2), :].reshape(CK // 16, 8, 128) & lm[None]
        return pltpu.bitcast(ki.reshape(CK // 2, 128), BF16)

    def qwin(h, js):
        return pltpu.bitcast(qt_ref[pl.ds(pl.multiple_of(window(h) * 32, 32), 64), cols(js)], BF16)

    def qk_chunk(kc, q, js, c):
        s = jnp.dot(kc, q, preferred_element_type=F32)
        s_ref[js, c * CK:(c + 1) * CK, :] = s
        return jnp.max(s.reshape(CK // 8, 8, TQ), axis=0)

    def pexp(js, c, m):
        return jnp.exp2(s_ref[js, c * CK:(c + 1) * CK, :] - m).astype(BF16)

    def pv_chunk(p, r0, ones_mask, c):
        v = jnp.where(ones_mask, 1.0, vt_ref[pl.ds(r0, 24), c * CK:(c + 1) * CK])
        return jnp.dot(v, p, preferred_element_type=F32)

    def head_rows(h):
        off = (h & 1) * 4
        if isinstance(h, int):
            return h * DH - off, off, (20 if off == 0 else 0)
        return pl.multiple_of(h * DH - off, 8), off, jnp.where(off == 0, 20, 0)

    def finish(acc, js, r0, off, ones_row):
        l = jnp.sum(jnp.where(row24q == ones_row, acc, 0.0), axis=0, keepdims=True)
        o = acc * (1.0 / l)
        keep = (row24q >= off) & (row24q < off + DH)
        pltpu.store(ot_ref.at[pl.ds(r0, 24), cols(js)], o, mask=keep)

    def qvproj(r, carry):
        rows = blk(r)
        prow = pl.ds(pl.multiple_of(r * (RB // 2), RB // 2), RB // 2)
        rolled = [pltpu.roll(kw_ref[2 * t, prow, :].reshape(RB // 16, 8, 128), 64, 2) for t in range(5)]
        for t in range(4):
            kw_ref[2 * t + 1, prow, :] = jnp.where(lo_half[None], rolled[t], rolled[t + 1]).reshape(RB // 2, 128)
        xn = pltpu.bitcast(xn_ref[prow, :], BF16)
        qv = lax.dot_general(wqvt_ref[...], xn, NT_DIMS, preferred_element_type=F32)
        qu = pltpu.bitcast((qv[0:D] * QSCALE).astype(BF16), U32)
        qt_ref[:, rows] = qu
        vt_ref[:, rows] = qv[D:2 * D].astype(BF16).astype(F32)
        q0 = pltpu.bitcast(qu[0:64], BF16)
        mx = None
        for c in range(NC):
            mc = qk_chunk(kmask(0, c), q0, r, c)
            mx = mc if mx is None else jnp.maximum(mx, mc)
        m_ref[:, rows] = jnp.broadcast_to(jnp.max(mx, axis=0, keepdims=True), (8, RB))
        return carry

    with jax.named_scope("qvproj"):
        lax.fori_loop(0, NRB, qvproj, 0)

    slots = [(js, c) for js in range(NS) for c in range(NC)]

    def finish_raw(hp):
        r0, off, ones_row = head_rows(hp)
        for js in range(NS):
            finish(acc_ref[js], js, r0, off, ones_row)

    def head_step(h, ms):
        r0, off, ones_row = head_rows(h)
        ones_mask = row24 == ones_row
        finish_raw(jnp.maximum(h - 1, 0))
        ks, mxs, accs = {}, {}, {}

        def do_qk(n):
            js, c = slots[n]
            if c not in ks:
                ks[c] = kmask(h + 1, c)
            mc = qk_chunk(ks[c], qwin(h + 1, js), js, c)
            mxs[js] = mc if c == 0 else jnp.maximum(mxs[js], mc)

        def do_pv(n, p):
            js, c = slots[n]
            d = pv_chunk(p, r0, ones_mask, c)
            accs[js] = d if c == 0 else accs[js] + d
            if c == NC - 1:
                acc_ref[js] = accs[js]

        p_next = pexp(0, 0, ms[0])
        do_qk(0)
        for n in range(len(slots)):
            p = p_next
            if n + 1 < len(slots):
                p_next = pexp(slots[n + 1][0], slots[n + 1][1], ms[slots[n + 1][0]])
                do_qk(n + 1)
            do_pv(n, p)
        return tuple(jnp.max(mxs[js], axis=0, keepdims=True) for js in range(NS))

    with jax.named_scope("attention"):
        ms = tuple(m_ref[0:1, js * TQ:(js + 1) * TQ] for js in range(NS))
        acc_ref[...] = jnp.ones(acc_ref.shape, F32)
        ms = lax.fori_loop(0, H - 1, head_step, ms)
        finish_raw(H - 2)

    r0_l, off_l, ones_l = head_rows(H - 1)
    m_ref[:, :] = jnp.broadcast_to(jnp.concatenate(ms, axis=1), (8, S))

    def pv_last(js, c, acc):
        d = pv_chunk(pexp(js, c, m_ref[0:1, cols(js)]), r0_l, row24 == ones_l, c)
        return d if acc is None else acc + d

    with jax.named_scope("last_head"):
        acc = None
        for c in range(NC):
            acc = pv_last(0, c, acc)
        finish(acc, 0, r0_l, off_l, ones_l)
        ob_ref[...] = pltpu.bitcast(ot_ref[:, 0:HR].astype(BF16).T, U32)
        for cp in late_copies:
            cp.wait()

    def half(r, i):
        return pl.ds(r * RB + i * HR if isinstance(r, int) else pl.multiple_of(r * RB + i * HR, HR), HR)

    def out_copy(r, i):
        return pltpu.make_async_copy(y_ref.at[half(r, i)], o_hbm.at[half(r, i)], out_sems.at[2 * r + i])

    def tail(r, carry):
        rn = jnp.minimum(r + 1, NRB - 1)
        os_ = [pltpu.bitcast(ob_ref[...], BF16), ot_ref[:, half(r, 1)].astype(BF16).T]
        hres = [x_ref[half(r, i), :].astype(F32) + jnp.dot(os_[i], wo_ref[...], preferred_element_type=F32)
                for i in range(2)]
        hn = [_ln(hh).astype(BF16) for hh in hres]
        acc = None
        c_pv = 0
        a = []
        for i in range(2):
            parts = []
            for (n0, nt) in GROUPS:
                g = lax.dot_general(hn[i], w13t_ref[n0 * 128:(n0 + nt) * 128, :], NT_DIMS,
                                    preferred_element_type=F32)
                u = lax.dot_general(hn[i], w13t_ref[FM + n0 * 128:FM + (n0 + nt) * 128, :], NT_DIMS,
                                    preferred_element_type=F32)
                parts.append((_silu(g) * u).astype(BF16))
                for _ in range(2):
                    acc = pv_last(rn, c_pv, acc)
                    c_pv += 1
            t = lax.dot_general(hn[i], w13t_ref[2 * FM:2 * F, :], NT_DIMS, preferred_element_type=F32)
            parts.append(jnp.where(lo_half[0:1], _silu(t) * pltpu.roll(t, 64, 1), 0.0).astype(BF16))
            a.append(jnp.concatenate(parts, axis=1))
        assert c_pv == NC
        finish(acc, rn, r0_l, off_l, ones_l)
        ob_ref[...] = pltpu.bitcast(ot_ref[:, half(rn, 0)].astype(BF16).T, U32)
        for i in range(2):
            y = hres[i] + jnp.dot(a[i], w2_ref[...], preferred_element_type=F32)
            y_ref[half(r, i), :] = y.astype(BF16)
            out_copy(r, i).start()
        return carry

    with jax.named_scope("ffn"):
        lax.fori_loop(0, NRB, tail, 0)
        for r in range(NRB):
            for i in range(2):
                out_copy(r, i).wait()


@jax.jit
def pallas_sequential_preLN__softmax_full_mha__glu_gated_swiglu__prompt_kernel(
    A_x: jax.Array,
    A_wqkv: jax.Array,
    A_wo: jax.Array,
    B_x: jax.Array,
    B_w1: jax.Array,
    B_w3: jax.Array,
    B_w2: jax.Array,
):
    del B_x
    hbm = pl.BlockSpec(memory_space=pltpu.HBM)
    out = pl.pallas_call(
        _kernel,
        out_shape=jax.ShapeDtypeStruct((S, D), BF16),
        in_specs=[hbm] * 6,
        out_specs=hbm,
        scratch_shapes=[
            pltpu.VMEM((S, D), BF16),
            pltpu.VMEM((D, 3 * D), BF16),
            pltpu.VMEM((D, D), BF16),
            pltpu.VMEM((2 * F, D), BF16),
            pltpu.VMEM((F + FT, D), BF16),
            pltpu.VMEM((S, D), BF16),
            pltpu.VMEM((S // 2, D), U32),
            pltpu.VMEM((2 * D, D), BF16),
            pltpu.VMEM((NW, S // 2, 128), U32),
            pltpu.VMEM((D // 2, S), U32),
            pltpu.VMEM((D, S), F32),
            pltpu.VMEM((NS, S, TQ), F32),
            pltpu.VMEM((D, S), F32),
            pltpu.VMEM((8, S), F32),
            pltpu.VMEM((NS, 24, TQ), F32),
            pltpu.VMEM((HR // 2, D), U32),
            pltpu.SemaphoreType.DMA((NRB,)),
            pltpu.SemaphoreType.DMA((9,)),
            pltpu.SemaphoreType.DMA((2 * NRB,)),
        ],
        compiler_params=pltpu.CompilerParams(vmem_limit_bytes=110 * 1024 * 1024),
        name="fused_block",
    )(A_x.reshape(S, D), A_wqkv, A_wo, B_w1.T, B_w3.T, B_w2)
    return out.reshape(1, S, D)
```

```python
import math

import jax
import jax.numpy as jnp
from jax import lax
import jax.experimental.pallas as pl
import jax.experimental.pallas.tpu as pltpu

S, D, H, DH, F = 2048, 640, 32, 20, 1728
NW = 9
CK = 128
NC = S // CK
TA = 256
NA = S // TA
SKEW = 2
RB = 512
NRB = S // RB
HR = RB // 2
FM = 1664
FT = F - FM
LNG = 16
EPS = 1e-5
LOG2E = float(math.log2(math.e))
GROUPS = ((0, 7), (7, 6))
QSCALE = float(DH ** -0.5 * math.log2(math.e))
NT_DIMS = (((1,), (1,)), ((), ()))
F32, BF16, U32 = jnp.float32, jnp.bfloat16, jnp.uint32


def _ln(x):
    mu = jnp.mean(x, axis=-1, keepdims=True)
    xc = x - mu
    var = jnp.mean(xc * xc, axis=-1, keepdims=True)
    return xc * lax.rsqrt(var + EPS)


def _silu(g):
    d = 1.0 + jnp.exp2(jnp.minimum(g * (-LOG2E), 126.0))
    r = pltpu.reciprocal(d, approx=True)
    return g * (r * (2.0 - d * r))


def _kernel(x_hbm, wqkv_hbm, wo_hbm, w1t_hbm, w3t_hbm, w2_hbm, o_hbm,
            x_ref, wqkv_ref, wo_ref, w13t_ref, w2_ref, y_ref,
            xn_ref, wqvt_ref, kw_ref, qt_ref, vt_ref, s_ref, ot_ref, m_ref, acc_ref, ob_ref,
            x_sems, w_sems, out_sems):
    def blk(r):
        return pl.ds(r * RB if isinstance(r, int) else pl.multiple_of(r * RB, RB), RB)

    def x_copy(r):
        return pltpu.make_async_copy(x_hbm.at[blk(r)], x_ref.at[blk(r)], x_sems.at[r])

    wk_copy = pltpu.make_async_copy(wqkv_hbm.at[:, D:2 * D], wqkv_ref.at[:, D:2 * D], w_sems.at[0])
    wq_copy = pltpu.make_async_copy(wqkv_hbm.at[:, 0:D], wqkv_ref.at[:, 0:D], w_sems.at[1])
    wv_copy = pltpu.make_async_copy(wqkv_hbm.at[:, 2 * D:3 * D], wqkv_ref.at[:, 2 * D:3 * D], w_sems.at[2])
    late_copies = [
        pltpu.make_async_copy(wo_hbm, wo_ref, w_sems.at[3]),
        pltpu.make_async_copy(w1t_hbm.at[0:FM], w13t_ref.at[0:FM], w_sems.at[4]),
        pltpu.make_async_copy(w3t_hbm.at[0:FM], w13t_ref.at[FM:2 * FM], w_sems.at[5]),
        pltpu.make_async_copy(w1t_hbm.at[FM:F], w13t_ref.at[2 * FM:2 * FM + FT], w_sems.at[6]),
        pltpu.make_async_copy(w3t_hbm.at[FM:F], w13t_ref.at[2 * FM + FT:2 * F], w_sems.at[7]),
        pltpu.make_async_copy(w2_hbm, w2_ref.at[0:F], w_sems.at[8]),
    ]
    x_copy(0).start()
    wk_copy.start()
    x_copy(1).start()
    x_copy(2).start()
    x_copy(3).start()
    wq_copy.start()
    wv_copy.start()

    lane = lax.broadcasted_iota(jnp.int32, (8, 128), 1)
    lo_half = lane < 64

    def ln_block(r):
        for g in range(RB // LNG):
            rows = pl.ds(r * RB + g * LNG, LNG)
            prows = pl.ds(r * (RB // 2) + g * (LNG // 2), LNG // 2)
            xn_ref[prows, :] = pltpu.bitcast(_ln(x_ref[rows, :].astype(F32)).astype(BF16), U32)

    def kproj(r):
        for i in range(4):
            prow = pl.ds(r * (RB // 2) + i * (RB // 8), RB // 8)
            k = jnp.dot(pltpu.bitcast(xn_ref[prow, :], BF16), wqkv_ref[:, D:2 * D], preferred_element_type=F32)
            ku = pltpu.bitcast(k.astype(BF16), U32)
            for t in range(5):
                kw_ref[2 * t, prow, :] = ku[:, t * 128:(t + 1) * 128]

    with jax.named_scope("ln_kproj"):
        x_copy(0).wait()
        ln_block(0)
        w2_ref[F:F + FT, :] = jnp.zeros((FT, D), BF16)
        wk_copy.wait()
        kproj(0)
        x_copy(1).wait()
        x_copy(2).wait()
        ln_block(1)
        kproj(1)
        ln_block(2)
        x_copy(3).wait()
        wq_copy.wait()
        wv_copy.wait()
        for cp in late_copies:
            cp.start()
        kproj(2)
        ln_block(3)
        kproj(3)
        wqvt_ref[0:D, :] = wqkv_ref[:, 0:D].T
        wqvt_ref[D:2 * D, :] = wqkv_ref[:, 2 * D:3 * D].T

    row24 = lax.broadcasted_iota(jnp.int32, (24, 128), 0)

    def qcols(i):
        return pl.ds(i * TA if isinstance(i, int) else pl.multiple_of(i * TA, TA), TA)

    def window(h):
        return jnp.minimum((h * DH) >> 6, NW - 1)

    def kmask(h, c):
        w = window(h)
        lo = h * DH - w * 64
        lm = jnp.where((lane >= lo) & (lane < lo + DH), U32(0xFFFFFFFF), U32(0))
        ki = kw_ref[w, c * (CK // 2):(c + 1) * (CK // 2), :].reshape(CK // 16, 8, 128) & lm[None]
        return pltpu.bitcast(ki.reshape(CK // 2, 128), BF16)

    def qwin(h, qs):
        return pltpu.bitcast(qt_ref[pl.ds(pl.multiple_of(window(h) * 32, 32), 64), qs], BF16)

    def qk_chunk(kc, q, qs, c):
        s = jnp.dot(kc, q, preferred_element_type=F32)
        s_ref[c * CK:(c + 1) * CK, qs] = s
        return jnp.max(s.reshape(CK // 8, 8, s.shape[1]), axis=0)

    def pexp(qs, c, m):
        return jnp.exp2(s_ref[c * CK:(c + 1) * CK, qs] - m).astype(BF16)

    def pv_chunk(p, r0, ones_mask, c):
        v = jnp.where(ones_mask, 1.0, vt_ref[pl.ds(r0, 24), c * CK:(c + 1) * CK])
        return jnp.dot(v, p, preferred_element_type=F32)

    def head_rows(h):
        off = (h & 1) * 4
        if isinstance(h, int):
            return h * DH - off, off, (20 if off == 0 else 0)
        return pl.multiple_of(h * DH - off, 8), off, jnp.where(off == 0, 20, 0)

    def finish(acc, qs, r0, off, ones_row):
        row = lax.broadcasted_iota(jnp.int32, acc.shape, 0)
        l = jnp.sum(jnp.where(row == ones_row, acc, 0.0), axis=0, keepdims=True)
        r = pltpu.reciprocal(l, approx=True)
        o = acc * (r * (2.0 - l * r))
        keep = (row >= off) & (row < off + DH)
        pltpu.store(ot_ref.at[pl.ds(r0, 24), qs], o, mask=keep)

    def qvproj(r, carry):
        rows = blk(r)
        prow = pl.ds(pl.multiple_of(r * (RB // 2), RB // 2), RB // 2)
        rolled = [pltpu.roll(kw_ref[2 * t, prow, :].reshape(RB // 16, 8, 128), 64, 2) for t in range(5)]
        for t in range(4):
            kw_ref[2 * t + 1, prow, :] = jnp.where(lo_half[None], rolled[t], rolled[t + 1]).reshape(RB // 2, 128)
        xn = pltpu.bitcast(xn_ref[prow, :], BF16)
        qv = lax.dot_general(wqvt_ref[...], xn, NT_DIMS, preferred_element_type=F32)
        qu = pltpu.bitcast((qv[0:D] * QSCALE).astype(BF16), U32)
        qt_ref[:, rows] = qu
        vt_ref[:, rows] = qv[D:2 * D].astype(BF16).astype(F32)
        q0 = pltpu.bitcast(qu[0:64], BF16)
        mx = None
        for c in range(NC):
            mc = qk_chunk(kmask(0, c), q0, rows, c)
            mx = mc if mx is None else jnp.maximum(mx, mc)
        m_ref[:, rows] = jnp.broadcast_to(jnp.max(mx, axis=0, keepdims=True), (8, RB))
        return carry

    with jax.named_scope("qvproj"):
        lax.fori_loop(0, NRB, qvproj, 0)

    slots = [(ja, c) for ja in range(NA) for c in range(NC)]

    def finish_raw(hp):
        r0, off, ones_row = head_rows(hp)
        for r in range(NRB):
            finish(acc_ref[:, blk(r)], blk(r), r0, off, ones_row)

    def head_step(h, ms):
        r0, off, ones_row = head_rows(h)
        ones_mask = row24 == ones_row
        finish_raw(jnp.maximum(h - 1, 0))
        mxs, accs = {}, {}

        def do_qk(n):
            ja, c = slots[n]
            mc = qk_chunk(kmask(h + 1, c), qwin(h + 1, qcols(ja)), qcols(ja), c)
            mxs[ja] = mc if c == 0 else jnp.maximum(mxs[ja], mc)

        def do_pv(n, p):
            ja, c = slots[n]
            d = pv_chunk(p, r0, ones_mask, c)
            accs[ja] = d if c == 0 else accs[ja] + d
            if c == NC - 1:
                acc_ref[:, qcols(ja)] = accs[ja]

        ps = {}
        n_qk = 0
        for n in range(len(slots)):
            while n_qk < min(len(slots), n + 1 + SKEW):
                ja, c = slots[n_qk]
                ps[n_qk] = pexp(qcols(ja), c, ms[ja])
                do_qk(n_qk)
                n_qk += 1
            do_pv(n, ps.pop(n))
        return tuple(jnp.max(mxs[ja], axis=0, keepdims=True) for ja in range(NA))

    with jax.named_scope("attention"):
        ms = tuple(m_ref[0:1, qcols(ja)] for ja in range(NA))
        acc_ref[...] = jnp.ones(acc_ref.shape, F32)
        ms = lax.fori_loop(0, H - 1, head_step, ms)
        finish_raw(H - 2)

    r0_l, off_l, ones_l = head_rows(H - 1)
    m_ref[:, :] = jnp.broadcast_to(jnp.concatenate(ms, axis=1), (8, S))
    NP = RB // TA

    def pv_last(r, n, acc):
        k, c = n // NC, n % NC
        qs = qcols(r * NP + k)
        d = pv_chunk(pexp(qs, c, m_ref[0:1, qs]), r0_l, row24 == ones_l, c)
        acc = d if c == 0 else acc + d
        if c == NC - 1:
            finish(acc, qs, r0_l, off_l, ones_l)
        return acc

    with jax.named_scope("last_head"):
        acc = None
        for n in range(NC * NP):
            acc = pv_last(0, n, acc)
        ob_ref[...] = pltpu.bitcast(ot_ref[:, 0:HR].astype(BF16).T, U32)
        for cp in late_copies:
            cp.wait()

    def half(r, i):
        return pl.ds(r * RB + i * HR if isinstance(r, int) else pl.multiple_of(r * RB + i * HR, HR), HR)

    PIECES = ((0, HR), (HR, HR // 2), (HR + HR // 2, HR // 2))

    def piece(r, i):
        start, size = PIECES[i]
        return pl.ds(r * RB + start if isinstance(r, int) else pl.multiple_of(r * RB + start, size), size)

    def out_copy(r, i):
        return pltpu.make_async_copy(y_ref.at[piece(r, i)], o_hbm.at[piece(r, i)], out_sems.at[3 * r + i])

    def tail(r, carry):
        rn = jnp.minimum(r + 1, NRB - 1)
        os_ = [pltpu.bitcast(ob_ref[...], BF16), ot_ref[:, half(r, 1)].astype(BF16).T]
        hres = [x_ref[half(r, i), :].astype(F32) + jnp.dot(os_[i], wo_ref[...], preferred_element_type=F32)
                for i in range(2)]
        hn = [_ln(hh).astype(BF16) for hh in hres]
        acc = None
        n_pv = 0
        a = []
        for i in range(2):
            parts = []
            for (n0, nt) in GROUPS:
                gu = []
                for base in (0, FM):
                    gu.append(lax.dot_general(hn[i], w13t_ref[base + n0 * 128:base + (n0 + nt) * 128, :], NT_DIMS,
                                              preferred_element_type=F32))
                    for _ in range(2 * NP):
                        acc = pv_last(rn, n_pv, acc)
                        n_pv += 1
                parts.append((_silu(gu[0]) * gu[1]).astype(BF16))
            t = lax.dot_general(hn[i], w13t_ref[2 * FM:2 * F, :], NT_DIMS, preferred_element_type=F32)
            parts.append(jnp.where(lo_half[0:1], _silu(t) * pltpu.roll(t, 64, 1), 0.0).astype(BF16))
            a.append(jnp.concatenate(parts, axis=1))
        assert n_pv == NC * NP
        ob_ref[...] = pltpu.bitcast(ot_ref[:, half(rn, 0)].astype(BF16).T, U32)
        y_ref[piece(r, 0), :] = (hres[0] + jnp.dot(a[0], w2_ref[...], preferred_element_type=F32)).astype(BF16)
        out_copy(r, 0).start()
        for i in (1, 2):
            sl = slice((i - 1) * (HR // 2), i * (HR // 2))
            y = hres[1][sl] + jnp.dot(a[1][sl], w2_ref[...], preferred_element_type=F32)
            y_ref[piece(r, i), :] = y.astype(BF16)
            out_copy(r, i).start()
        return carry

    with jax.named_scope("ffn"):
        lax.fori_loop(0, NRB, tail, 0)
        for r in range(NRB):
            for i in range(3):
                out_copy(r, i).wait()


@jax.jit
def pallas_sequential_preLN__softmax_full_mha__glu_gated_swiglu__prompt_kernel(
    A_x: jax.Array,
    A_wqkv: jax.Array,
    A_wo: jax.Array,
    B_x: jax.Array,
    B_w1: jax.Array,
    B_w3: jax.Array,
    B_w2: jax.Array,
):
    del B_x
    hbm = pl.BlockSpec(memory_space=pltpu.HBM)
    out = pl.pallas_call(
        _kernel,
        out_shape=jax.ShapeDtypeStruct((S, D), BF16),
        in_specs=[hbm] * 6,
        out_specs=hbm,
        scratch_shapes=[
            pltpu.VMEM((S, D), BF16),
            pltpu.VMEM((D, 3 * D), BF16),
            pltpu.VMEM((D, D), BF16),
            pltpu.VMEM((2 * F, D), BF16),
            pltpu.VMEM((F + FT, D), BF16),
            pltpu.VMEM((S, D), BF16),
            pltpu.VMEM((S // 2, D), U32),
            pltpu.VMEM((2 * D, D), BF16),
            pltpu.VMEM((NW, S // 2, 128), U32),
            pltpu.VMEM((D // 2, S), U32),
            pltpu.VMEM((D, S), F32),
            pltpu.VMEM((S, S), F32),
            pltpu.VMEM((D, S), F32),
            pltpu.VMEM((8, S), F32),
            pltpu.VMEM((24, S), F32),
            pltpu.VMEM((HR // 2, D), U32),
            pltpu.SemaphoreType.DMA((NRB,)),
            pltpu.SemaphoreType.DMA((9,)),
            pltpu.SemaphoreType.DMA((3 * NRB,)),
        ],
        compiler_params=pltpu.CompilerParams(vmem_limit_bytes=110 * 1024 * 1024),
        name="fused_block",
    )(A_x.reshape(S, D), A_wqkv, A_wo, B_w1.T, B_w3.T, B_w2)
    return out.reshape(1, S, D)
```
